```python
import jax
import jax.numpy as jnp

def _softmax(x, axis=-1):
    return jax.nn.softmax(x, axis=axis)
def _gelu(x):
    return jax.nn.gelu(x, approximate=True)
def _silu(x):
    return jax.nn.silu(x)
def _sigmoid(x):
    return jax.nn.sigmoid(x)
def _layernorm(x, axis=-1, eps=1e-5):
    m = jnp.mean(x, axis=axis, keepdims=True)
    v = jnp.var(x, axis=axis, keepdims=True)
    return (x - m) / jnp.sqrt(v + eps)
def _scatter_add(tgt, idx, src, axis=0):
    return tgt.at[idx].add(src)
def _segment_sum(src, seg, n):
    return jax.ops.segment_sum(src, seg, n)
class _Rng:
    def __init__(self, key):
        self._k = key
    def _next(self):
        self._k, sub = jax.random.split(self._k)
        return sub
    def normal(self, shape):
        return jax.random.normal(self._next(), shape, dtype=jnp.bfloat16)
    def randint(self, lo, hi, shape):
        return jax.random.randint(self._next(), shape, lo, hi, dtype=jnp.int32)
    def uniform(self, shape, lo=0.0, hi=1.0):
        return jax.random.uniform(self._next(), shape, jnp.bfloat16, lo, hi)
    def permutation(self, n):
        return jax.random.permutation(self._next(), n)


kernel_name = 'sequential_preLN__linear_attn_block__moe_arch_mod__prompt'

def setup_inputs():
    _rng = _Rng(jax.random.key(int.from_bytes(__import__("os").urandom(4), "little")))
    _w = (lambda a: (lambda t: t.astype(jnp.bfloat16) if jnp.issubdtype(t.dtype, jnp.floating) else t)(jnp.asarray(a)))
    def _A_setup():
        B, S, D = 1, 2048, 1024
        return {
            "x": _w((lambda *s: _rng.normal(s) * 0.05)(B, S, D)),
            "wqkv": _w((lambda *s: _rng.normal(s) * 0.05)(D, 3 * D)),
            "wo": _w((lambda *s: _rng.normal(s) * 0.05)(D, D)),
        }
    _A_in = _A_setup()

    def _B_setup():
        B, S, D, F, C = 1, 2048, 1024, 3584, 2
        return {
            "x": _w((lambda *s: _rng.normal(s) * 0.05)(B, S, D)),
            "w_r": _w((lambda *s: _rng.normal(s) * 0.05)(D)),
            "w_gate": _w((lambda *s: _rng.normal(s) * 0.05)(D, F)),
            "w_up": _w((lambda *s: _rng.normal(s) * 0.05)(D, F)),
            "w_down": _w((lambda *s: _rng.normal(s) * 0.05)(F, D)),
        }
    _B_in = _B_setup()

    return {
        "A_x": _A_in["x"],
        "A_wqkv": _A_in["wqkv"],
        "A_wo": _A_in["wo"],
        "B_x": _B_in["x"],
        "B_w_r": _B_in["w_r"],
        "B_w_gate": _B_in["w_gate"],
        "B_w_up": _B_in["w_up"],
        "B_w_down": _B_in["w_down"],
    }

def reference(A_x, A_wqkv, A_wo, B_x, B_w_r, B_w_gate, B_w_up, B_w_down):
    def _A_ref(x, wqkv, wo):
        B, S, D = x.shape
        H = 32; Dh = D // H
        qkv = (lambda x, *d: x.transpose(*d))((x @ wqkv).reshape(B, S, 3, H, Dh), 2, 0, 3, 1, 4)
        q, k, v = qkv[0], qkv[1], qkv[2]
        phi = lambda t: jnp.where(t > 0, t + 1, jnp.exp(t)) + 1e-6
        pq, pk = phi(q), phi(k)
        kv = jnp.einsum("bhsd,bhse->bhde", pk, v)
        z = jnp.einsum("bhsd->bhd", pk)
        num = jnp.einsum("bhqd,bhde->bhqe", pq, kv)
        den = jnp.einsum("bhqd,bhd->bhq", pq, z)[..., None] + 1e-6
        o = num / den
        return (lambda x, *d: x.transpose(*d))(o, 0, 2, 1, 3).reshape(B, S, D) @ wo

    def _B_ref(x, w_r, w_gate, w_up, w_down):
        B, S, D = x.shape
        C = 2
        r = x @ w_r
        idx = jnp.argsort(-r, axis=-1)[:, :C]
        idx_e = jnp.repeat(idx.reshape(B, C, 1), D, axis=2)
        x_sel = jnp.take_along_axis(x, idx_e, axis=1)
        g = _silu(x_sel @ w_gate)
        u = x_sel @ w_up
        y = (g * u) @ w_down
        r_sel = _sigmoid(jnp.take_along_axis(r, idx, axis=1))
        y = y * r_sel.reshape(B, C, 1)
        b_off = (jnp.arange(B) * S).reshape(B, 1)
        flat_idx = (idx + b_off).reshape(B * C)
        zero = (x * 0.0).reshape(B * S, D)
        upd = _scatter_add(zero, flat_idx, y.reshape(B * C, D), axis=0)
        return x + upd.reshape(B, S, D)

    x = A_x
    h = x + _A_ref(_layernorm(x, axis=-1), A_wqkv, A_wo)
    h2 = h + _B_ref(_layernorm(h, axis=-1), B_w_r, B_w_gate, B_w_up, B_w_down)
    return h2
```

```python
import jax
import jax.numpy as jnp
import jax.experimental.pallas as pl
import jax.experimental.pallas.tpu as pltpu

F32 = jnp.float32
BF16 = jnp.bfloat16
H = 32
T = 256
LANES = 128
NB2 = 1024
NB1 = 256
EPS_LN = 1e-5
EPS_ATT = 1e-6


def _ln(x):
    m = jnp.mean(x, axis=-1, keepdims=True)
    xc = x - m
    v = jnp.mean(xc * xc, axis=-1, keepdims=True)
    return xc * jax.lax.rsqrt(v + EPS_LN)


def _phi(t):
    return jnp.where(t > 0, t + 1.0, jnp.exp(t)) + EPS_ATT


def _dot(a, b):
    return jnp.dot(a, b, preferred_element_type=F32)


def _kernel(x_hbm, wqkv_hbm, wo_hbm, wr_hbm, wg_hbm, wu_hbm, wd_hbm, out_hbm,
            x_v, st_v, cs_v, wqkv_v, wo_v, wr_v, wg_v, wu_v, wd_v, kv_acc, z_acc, m_v, zc_v, o_v,
            out_v, h_v, r_v, fix_v, x_sems, w_sems, in_sems, out_sems, fix_sems):
    S, D = x_v.shape
    nt = S // T
    dh = D // H
    G = D // LANES
    NB = NB1
    nb = D // NB

    def x_copy(i):
        return pltpu.make_async_copy(x_hbm.at[pl.ds(i * T, T)], x_v.at[pl.ds(i * T, T)], x_sems.at[i])

    def w_copy(j):
        c = pl.ds(D + (j % 2) * D + (j // 2) * NB, NB)
        return pltpu.make_async_copy(wqkv_hbm.at[:, c], wqkv_v.at[:, c], w_sems.at[j])

    cp_wq = pltpu.make_async_copy(wqkv_hbm.at[:, pl.ds(0, D)], wqkv_v.at[:, pl.ds(0, D)], in_sems.at[0])
    cp_wo = pltpu.make_async_copy(wo_hbm, wo_v, in_sems.at[1])
    cp_wg = pltpu.make_async_copy(wg_hbm, wg_v, in_sems.at[2])
    cp_wu = pltpu.make_async_copy(wu_hbm, wu_v, in_sems.at[3])
    cp_wd = pltpu.make_async_copy(wd_hbm, wd_v, in_sems.at[4])
    cp_wr = pltpu.make_async_copy(wr_hbm, wr_v, in_sems.at[5])

    x_copy(0).start()
    w_copy(0).start()
    w_copy(1).start()
    kv_acc[...] = jnp.zeros(kv_acc.shape, F32)
    z_acc[...] = jnp.zeros(z_acc.shape, F32)
    r_v[...] = jnp.zeros(r_v.shape, F32)

    def stats(i):
        r0 = pl.multiple_of(i * T, T)
        x = x_v[pl.ds(r0, T), :].astype(F32)
        m = jnp.mean(x, axis=-1, keepdims=True)
        xc = x - m
        v = jnp.mean(xc * xc, axis=-1, keepdims=True)
        s = jax.lax.rsqrt(v + EPS_LN)
        st_v[0, pl.ds(r0, T), :] = jnp.broadcast_to(s, (T, LANES))
        st_v[1, pl.ds(r0, T), :] = jnp.broadcast_to(m * s, (T, LANES))

    def colsum(c0, NB=NB1):
        w = wqkv_v[:, c0:c0 + NB].astype(F32)
        cs_v[:, c0:c0 + NB] = jnp.broadcast_to(jnp.sum(w, axis=0, keepdims=True), (8, NB))

    def proj(i, c0, NB=NB2):
        r0 = pl.multiple_of(i * T, T)
        acc = _dot(x_v[pl.ds(r0, T), :], wqkv_v[:, c0:c0 + NB])
        rep = NB // LANES
        s = jnp.concatenate([st_v[0, pl.ds(r0, T), :]] * rep, axis=1)
        ms = jnp.concatenate([st_v[1, pl.ds(r0, T), :]] * rep, axis=1)
        c = jnp.broadcast_to(cs_v[:, c0:c0 + NB][None], (T // 8, 8, NB)).reshape(T, NB)
        return acc * s - ms * c

    x_copy(0).wait()

    def p1(i, first):
        r0 = pl.multiple_of(i * T, T)
        NB = NB1 if first else NB2
        nb = D // NB
        if first:
            stats(i)

        def kv_update(b, pkb, vb):
            z_acc[:, b * NB:(b + 1) * NB] += jnp.sum(pkb.astype(F32).reshape(T // 8, 8, NB), axis=0)
            for g in range(NB // LANES):
                sl = slice(g * LANES, (g + 1) * LANES)
                kv_acc[b * (NB // LANES) + g] += jax.lax.dot_general(
                    pkb[:, sl], vb[:, sl], (((0,), (0,)), ((), ())), preferred_element_type=F32)

        prev = None
        for b in range(nb):
            if first:
                w_copy(2 * b).wait()
                if b == 1:
                    x_copy(1).start()
                if 2 * b + 2 < 2 * nb:
                    w_copy(2 * b + 2).start()
                colsum(D + b * NB)
            k = proj(i, D + b * NB, NB)
            if first:
                w_copy(2 * b + 1).wait()
                if 2 * b + 3 < 2 * nb:
                    w_copy(2 * b + 3).start()
            if prev is not None:
                kv_update(*prev)
            if first:
                colsum(2 * D + b * NB)
            vb = proj(i, 2 * D + b * NB, NB).astype(BF16)
            pkb = _phi(k).astype(BF16)
            prev = (b, pkb, vb)
        if first:
            for t in range(2, nt):
                x_copy(t).start()
            cp_wq.start()
            cp_wo.start()
            cp_wr.start()
        if first:
            x_copy(1).wait()
        stats(jnp.minimum(i + 1, nt - 1))
        kv_update(*prev)

    p1(0, True)

    def p1_loop(i, c):
        @pl.when(i + 1 < nt)
        def _():
            x_copy(i + 1).wait()

        @pl.when(i == 1)
        def _():
            cp_wg.start()

        @pl.when(i == 3)
        def _():
            cp_wu.start()

        @pl.when(i == 5)
        def _():
            cp_wd.start()
        p1(i, False)
        return c

    jax.lax.fori_loop(1, nt, p1_loop, 0)

    cp_wo.wait()
    cp_wq.wait()
    cp_wr.wait()
    for b in range(nb):
        colsum(b * NB)
    ri = jax.lax.broadcasted_iota(jnp.int32, (LANES, LANES), 0) // dh
    ci = jax.lax.broadcasted_iota(jnp.int32, (LANES, LANES), 1) // dh
    blk = ri == ci
    z = jnp.sum(z_acc[...], axis=0, keepdims=True).astype(BF16).astype(F32)
    for g in range(G):
        sl = slice(g * LANES, (g + 1) * LANES)
        zc_v[sl, :] = jnp.broadcast_to(z[:, sl], (LANES, LANES)).T
    for g in range(G):
        sl = slice(g * LANES, (g + 1) * LANES)
        kvg = jnp.where(blk, kv_acc[g], 0.0).astype(BF16)
        m_v[sl, :] = _dot(kvg, wo_v[sl, :]).astype(BF16)

    nb2 = D // NB2
    lane = jax.lax.broadcasted_iota(jnp.int32, (8, S // 8), 1)

    def out_copy(i):
        return pltpu.make_async_copy(out_v.at[pl.ds(i * T, T)], out_hbm.at[pl.ds(i * T, T)], out_sems.at[i])

    def q_dot(i, b):
        return proj(i, b * NB2)

    def q_post(i, b, q):
        pqt = _phi(q).astype(BF16).T.astype(F32)
        os_ = []
        for h in range(NB2 // dh):
            p = pqt[h * dh:(h + 1) * dh, :]
            zc = zc_v[b * NB2 + h * dh:b * NB2 + (h + 1) * dh, :]
            den = jnp.sum(p * jnp.concatenate([zc] * (T // LANES), axis=1), axis=0, keepdims=True) + EPS_ATT
            os_.append((p * (1.0 / den)).astype(BF16))
        o_v[i % 2, :, b * NB2:(b + 1) * NB2] = jnp.concatenate(os_, axis=0).T

    def stage_o(i, n):
        r0 = pl.multiple_of(i * T, T)
        cs = slice(n * NB2, (n + 1) * NB2)
        h_v[pl.ds(r0, T), cs] = x_v[pl.ds(r0, T), cs].astype(F32) + _dot(o_v[i % 2], m_v[:, cs])

    def stage_e(i, c, n):
        tc = T // n
        r0 = pl.multiple_of(i * T + c * tc, tc)
        h = h_v[pl.ds(r0, tc), :]
        hn = _ln(h)
        out_v[pl.ds(r0, tc), :] = (h + hn).astype(BF16)
        wr = wr_v[...].astype(F32).reshape(1, D)
        r = jnp.sum(hn * wr, axis=-1, keepdims=True)
        acc = r_v[...]
        for j in range(tc // 8):
            acc = jnp.where(lane == (i * T + c * tc) // 8 + j, r[j * 8:(j + 1) * 8, :], acc)
        r_v[...] = acc

    def body(i, do_q, do_o, do_e):
        prev = None
        if do_q:
            for b in range(nb2):
                q = q_dot(i + 1, b)
                if prev is not None:
                    q_post(i + 1, *prev)
                if do_e:
                    stage_e(i - 1, b, nb2)
                prev = (b, q)
        elif do_e and not do_o:
            stage_e(i - 1, 0, 1)
        if do_o:
            for n in range(nb2):
                stage_o(i, n)
                if n == 0 and prev is not None:
                    q_post(i + 1, *prev)
                    prev = None
                if do_e and not do_q:
                    stage_e(i - 1, n, nb2)
        if prev is not None:
            q_post(i + 1, *prev)
        if do_e:
            out_copy(i - 1).start()

    body(-1, True, False, False)
    body(0, True, True, False)

    def p2(i, c):
        body(i, True, True, True)
        return c

    jax.lax.fori_loop(1, nt - 1, p2, 0)
    body(nt - 1, False, True, True)
    body(nt, False, False, True)

    r = r_v[...]
    tok = lane * 8 + jax.lax.broadcasted_iota(jnp.int32, (8, S // 8), 0)
    m1 = jnp.max(r)
    i1 = jnp.min(jnp.where(r == m1, tok, S - 1))
    r2 = jnp.where(tok == i1, -jnp.inf, r)
    m2 = jnp.max(r2)
    i2 = jnp.min(jnp.where((r2 == m2) & (tok != i1), tok, S - 1))
    i1 = jnp.clip(i1, 0, S - 1)
    i2 = jnp.clip(i2, 0, S - 1)

    row = jax.lax.broadcasted_iota(jnp.int32, (16, 1), 0)
    xs = jnp.where(row == 0, h_v[pl.ds(i1, 1), :], jnp.where(row == 1, h_v[pl.ds(i2, 1), :], 0.0))
    xs = _ln(xs).astype(BF16)
    cp_wg.wait()
    cp_wu.wait()
    cp_wd.wait()
    acts = []
    for j in range(wg_v.shape[1] // LANES):
        cs = slice(j * LANES, (j + 1) * LANES)
        gate = _dot(xs, wg_v[:, cs])
        up = _dot(xs, wu_v[:, cs])
        acts.append((gate * jax.nn.sigmoid(gate) * up).astype(BF16))
    act = jnp.concatenate(acts, axis=1)
    y = jnp.concatenate([_dot(act, wd_v[:, j * LANES:(j + 1) * LANES]) for j in range(G)], axis=1)
    y1 = y[0:1, :] * jax.nn.sigmoid(jnp.full((1, LANES), m1, F32))[:, 0:1]
    y2 = y[1:2, :] * jax.nn.sigmoid(jnp.full((1, LANES), m2, F32))[:, 0:1]

    b1 = pl.multiple_of((i1 // 16) * 16, 16)
    b2 = pl.multiple_of((i2 // 16) * 16, 16)

    def fixed(b):
        h2 = out_v[pl.ds(b, 16), :].astype(F32)
        t = row + b
        upd = jnp.where(t == i1, y1, 0.0) + jnp.where(t == i2, y2, 0.0)
        return (h2 + upd).astype(BF16)

    fix_v[0] = fixed(b1)
    fix_v[1] = fixed(b2)
    for i in range(nt):
        out_copy(i).wait()
    c1 = pltpu.make_async_copy(fix_v.at[0], out_hbm.at[pl.ds(b1, 16)], fix_sems.at[0])
    c2 = pltpu.make_async_copy(fix_v.at[1], out_hbm.at[pl.ds(b2, 16)], fix_sems.at[1])
    c1.start()

    @pl.when(b1 != b2)
    def _():
        c2.start()
        c2.wait()

    c1.wait()


@jax.jit
def pallas_sequential_preLN__linear_attn_block__moe_arch_mod__prompt_kernel(
        A_x, A_wqkv, A_wo, B_x, B_w_r, B_w_gate, B_w_up, B_w_down):
    del B_x
    B, S, D = A_x.shape
    Fd = B_w_gate.shape[1]
    nt = S // T
    any_spec = pl.BlockSpec(memory_space=pl.ANY)
    out = pl.pallas_call(
        _kernel,
        in_specs=[any_spec] * 7,
        out_specs=any_spec,
        out_shape=jax.ShapeDtypeStruct((S, D), A_x.dtype),
        scratch_shapes=[
            pltpu.VMEM((S, D), BF16),
            pltpu.VMEM((2, S, LANES), F32),
            pltpu.VMEM((8, 3 * D), F32),
            pltpu.VMEM((D, 3 * D), BF16),
            pltpu.VMEM((D, D), BF16),
            pltpu.VMEM((D,), BF16),
            pltpu.VMEM((D, Fd), BF16),
            pltpu.VMEM((D, Fd), BF16),
            pltpu.VMEM((Fd, D), BF16),
            pltpu.VMEM((D // LANES, LANES, LANES), F32),
            pltpu.VMEM((8, D), F32),
            pltpu.VMEM((D, D), BF16),
            pltpu.VMEM((D, LANES), F32),
            pltpu.VMEM((2, T, D), BF16),
            pltpu.VMEM((S, D), BF16),
            pltpu.VMEM((S, D), F32),
            pltpu.VMEM((8, S // 8), F32),
            pltpu.VMEM((2, 16, D), BF16),
            pltpu.SemaphoreType.DMA((nt,)),
            pltpu.SemaphoreType.DMA((2 * D // NB1,)),
            pltpu.SemaphoreType.DMA((6,)),
            pltpu.SemaphoreType.DMA((nt,)),
            pltpu.SemaphoreType.DMA((2,)),
        ],
        compiler_params=pltpu.CompilerParams(vmem_limit_bytes=100 * 1024 * 1024),
    )(A_x.reshape(S, D), A_wqkv, A_wo, B_w_r, B_w_gate, B_w_up, B_w_down)
    return out.reshape(B, S, D)
```

```python
import jax
import jax.numpy as jnp
import jax.experimental.pallas as pl
import jax.experimental.pallas.tpu as pltpu

F32 = jnp.float32
BF16 = jnp.bfloat16
H = 32
T = 256
LANES = 128
PB = 256
NB2 = 1024
NB1 = 256
EPS_LN = 1e-5
EPS_ATT = 1e-6


def _ln(x):
    m = jnp.mean(x, axis=-1, keepdims=True)
    xc = x - m
    v = jnp.mean(xc * xc, axis=-1, keepdims=True)
    return xc * jax.lax.rsqrt(v + EPS_LN)


def _phi(t):
    return jnp.where(t > 0, t + 1.0, jnp.exp(t)) + EPS_ATT


def _dot(a, b):
    return jnp.dot(a, b, preferred_element_type=F32)


def _kernel(x_hbm, wqkv_hbm, wo_hbm, wr_hbm, wg_hbm, wu_hbm, wd_hbm, out_hbm,
            x_v, st_v, cs_v, wqkv_v, wo_v, wr_v, wg_v, wu_v, wd_v, pkt_v, p_v, z_acc, m_v, zc_v, o_v,
            out_v, h0_v, h1_v, r_v, fix_v, x_sems, w_sems, in_sems, out_sems, fix_sems):
    S, D = x_v.shape
    h_v = (h0_v, h1_v)
    nt = S // T
    dh = D // H
    G = D // LANES
    NB = NB1
    nb = D // NB

    def x_copy(i):
        return pltpu.make_async_copy(x_hbm.at[pl.ds(i * T, T)], x_v.at[pl.ds(i * T, T)], x_sems.at[i])

    def w_copy(j):
        c = pl.ds((1 - j % 2) * D + (j // 2) * NB, NB)
        return pltpu.make_async_copy(wqkv_hbm.at[:, c], wqkv_v.at[:, c], w_sems.at[j])

    cp_wv = pltpu.make_async_copy(wqkv_hbm.at[:, pl.ds(2 * D, D)], wqkv_v.at[:, pl.ds(2 * D, D)], in_sems.at[0])
    cp_wo = pltpu.make_async_copy(wo_hbm, wo_v, in_sems.at[1])
    class _Cols:
        def __init__(self, src, dst, sem):
            self.c = [pltpu.make_async_copy(src.at[:, pl.ds(j * LANES, LANES)], dst.at[j], sem)
                      for j in range(dst.shape[0])]

        def start(self):
            for c in self.c:
                c.start()

        def wait(self):
            for c in self.c:
                c.wait()

    cp_wg = _Cols(wg_hbm, wg_v, in_sems.at[2])
    cp_wu = _Cols(wu_hbm, wu_v, in_sems.at[3])
    cp_wd = _Cols(wd_hbm, wd_v, in_sems.at[4])
    cp_wr = pltpu.make_async_copy(wr_hbm, wr_v, in_sems.at[5])

    x_copy(0).start()
    w_copy(0).start()
    w_copy(1).start()
    z_acc[...] = jnp.zeros(z_acc.shape, F32)
    r_v[...] = jnp.zeros(r_v.shape, F32)

    def stats(i):
        r0 = pl.multiple_of(i * T, T)
        x = x_v[pl.ds(r0, T), :].astype(F32)
        m = jnp.mean(x, axis=-1, keepdims=True)
        xc = x - m
        v = jnp.mean(xc * xc, axis=-1, keepdims=True)
        s = jax.lax.rsqrt(v + EPS_LN)
        st_v[0, pl.ds(r0, T), :] = jnp.broadcast_to(s, (T, LANES))
        st_v[1, pl.ds(r0, T), :] = jnp.broadcast_to(m * s, (T, LANES))
        st_v[2, pl.ds(r0, T), :] = jnp.broadcast_to(m, (T, LANES))

    def colsum(c0, NB=NB1):
        w = wqkv_v[:, c0:c0 + NB].astype(F32)
        cs_v[:, c0:c0 + NB] = jnp.broadcast_to(jnp.sum(w, axis=0, keepdims=True), (8, NB))

    def proj(i, c0, NB=NB2):
        r0 = pl.multiple_of(i * T, T)
        acc = _dot(x_v[pl.ds(r0, T), :], wqkv_v[:, c0:c0 + NB])
        rep = NB // LANES
        s = jnp.concatenate([st_v[0, pl.ds(r0, T), :]] * rep, axis=1)
        ms = jnp.concatenate([st_v[1, pl.ds(r0, T), :]] * rep, axis=1)
        c = jnp.broadcast_to(cs_v[:, c0:c0 + NB][None], (T // 8, 8, NB)).reshape(T, NB)
        return acc * s - ms * c

    x_copy(0).wait()

    def pa(i, first):
        r0 = pl.multiple_of(i * T, T)
        NB = NB1 if first else NB2
        nb = D // NB
        if first:
            stats(i)
        for b in range(nb):
            cs = slice(b * NB, (b + 1) * NB)
            if first:
                w_copy(2 * b).wait()
                if b == 1:
                    x_copy(1).start()
                if 2 * b + 2 < 2 * nb:
                    w_copy(2 * b + 2).start()
                colsum(D + b * NB)
            pk = _phi(proj(i, D + b * NB, NB))
            if first:
                w_copy(2 * b + 1).wait()
                if 2 * b + 3 < 2 * nb:
                    w_copy(2 * b + 3).start()
                colsum(b * NB)
            rep = NB // LANES
            z_acc[0, :, cs] += jnp.sum(pk.astype(BF16).astype(F32).reshape(T // 8, 8, NB), axis=0)
            pks = (pk * jnp.concatenate([st_v[0, pl.ds(r0, T), :]] * rep, axis=1)).astype(BF16)
            mu = jnp.concatenate([st_v[2, pl.ds(r0, T), :]] * rep, axis=1)
            z_acc[1, :, cs] += jnp.sum((pks.astype(F32) * mu).reshape(T // 8, 8, NB), axis=0)
            pkt_v[cs, pl.ds(r0, T)] = pks.T
            o_v[pl.ds(r0, T), cs] = _phi(proj(i, b * NB, NB)).astype(BF16)
        if first:
            for t in range(2, nt):
                x_copy(t).start()
            cp_wv.start()
            cp_wo.start()
            cp_wr.start()
            x_copy(1).wait()
        stats(jnp.minimum(i + 1, nt - 1))

    pa(0, True)

    def pa_loop(i, c):
        @pl.when(i + 1 < nt)
        def _():
            x_copy(i + 1).wait()

        @pl.when(i == 1)
        def _():
            cp_wg.start()

        @pl.when(i == 3)
        def _():
            cp_wu.start()

        @pl.when(i == 5)
        def _():
            cp_wd.start()
        pa(i, False)
        return c

    jax.lax.fori_loop(1, nt, pa_loop, 0)

    cp_wo.wait()
    cp_wv.wait()
    cp_wr.wait()
    ri = jax.lax.broadcasted_iota(jnp.int32, (LANES, LANES), 0) // dh
    ci = jax.lax.broadcasted_iota(jnp.int32, (LANES, LANES), 1) // dh
    blk = ri == ci
    for w in range(2):
        z = jnp.sum(z_acc[w], axis=0, keepdims=True)
        if w == 0:
            z = z.astype(BF16).astype(F32)
        for g in range(G):
            sl = slice(g * LANES, (g + 1) * LANES)
            zc_v[w, sl, :] = jnp.broadcast_to(z[:, sl], (LANES, LANES)).T

    def stage_n(i):
        r0 = pl.multiple_of(i * T, T)
        for g in range(G):
            cs = slice(g * LANES, (g + 1) * LANES)
            pqt = o_v[pl.ds(r0, T), cs].T.astype(F32)
            os_ = []
            for h in range(LANES // dh):
                p = pqt[h * dh:(h + 1) * dh, :]
                zc = zc_v[0, g * LANES + h * dh:g * LANES + (h + 1) * dh, :]
                den = jnp.sum(p * jnp.concatenate([zc] * (T // LANES), axis=1), axis=0, keepdims=True) + EPS_ATT
                os_.append((p * (1.0 / den)).astype(BF16))
            o_v[pl.ds(r0, T), cs] = jnp.concatenate(os_, axis=0).T

    def stage_km(g):
        r0 = pl.multiple_of(g * LANES, LANES)
        kv = _dot(p_v[pl.ds(r0, LANES), :], wqkv_v[:, pl.ds(2 * D + r0, LANES)])
        kvg = jnp.where(blk, kv, 0.0).astype(BF16)
        m_v[pl.ds(r0, LANES), :] = _dot(kvg, wo_v[pl.ds(r0, LANES), :]).astype(BF16)

    def pb(j, km):
        r0 = pl.multiple_of(j * PB, PB)
        u = zc_v[1, pl.ds(r0, PB), :]
        p = _dot(pkt_v[pl.ds(r0, PB), :], x_v[...])
        p_v[pl.ds(r0, PB), :] = (p - jnp.concatenate([u] * G, axis=1)).astype(BF16)
        for t in range(nt * PB // D):
            stage_n(j * (nt * PB // D) + t)
        if km:
            for g in range(PB // LANES):
                stage_km((j - 1) * (PB // LANES) + g)

    pb(0, False)

    def pb_loop(j, c):
        pb(j, True)
        return c

    jax.lax.fori_loop(1, D // PB, pb_loop, 0)
    for g in range(PB // LANES):
        stage_km(G - PB // LANES + g)

    lane = jax.lax.broadcasted_iota(jnp.int32, (8, S // 8), 1)

    def out_copy(i):
        return pltpu.make_async_copy(out_v.at[pl.ds(i * T, T)], out_hbm.at[pl.ds(i * T, T)], out_sems.at[i])

    def stage_o(i, par):
        r0 = pl.multiple_of(i * T, T)
        q0 = pl.multiple_of((i // 2) * T, T)
        h_v[par][pl.ds(q0, T), :] = x_v[pl.ds(r0, T), :].astype(F32) + _dot(o_v[pl.ds(r0, T), :], m_v[...])

    def stage_e(i, par):
        r0 = pl.multiple_of(i * T, T)
        q0 = pl.multiple_of((i // 2) * T, T)
        h = h_v[par][pl.ds(q0, T), :]
        hn = _ln(h)
        out_v[pl.ds(r0, T), :] = (h + hn).astype(BF16)
        wr = wr_v[...].astype(F32).reshape(1, D)
        r = jnp.sum(hn * wr, axis=-1, keepdims=True)
        acc = r_v[...]
        for j in range(T // 8):
            acc = jnp.where(lane == i * (T // 8) + j, r[j * 8:(j + 1) * 8, :], acc)
        r_v[...] = acc
        out_copy(i).start()

    stage_o(0, 0)

    def pc(j, c):
        stage_e(2 * j, 0)
        stage_o(2 * j + 1, 1)
        stage_e(2 * j + 1, 1)
        stage_o(2 * j + 2, 0)
        return c

    jax.lax.fori_loop(0, nt // 2 - 1, pc, 0)
    stage_e(nt - 2, 0)
    stage_o(nt - 1, 1)
    stage_e(nt - 1, 1)

    r = r_v[...]
    tok = lane * 8 + jax.lax.broadcasted_iota(jnp.int32, (8, S // 8), 0)
    m1 = jnp.max(r)
    i1 = jnp.min(jnp.where(r == m1, tok, S - 1))
    r2 = jnp.where(tok == i1, -jnp.inf, r)
    m2 = jnp.max(r2)
    i2 = jnp.min(jnp.where((r2 == m2) & (tok != i1), tok, S - 1))
    i1 = jnp.clip(i1, 0, S - 1)
    i2 = jnp.clip(i2, 0, S - 1)

    row = jax.lax.broadcasted_iota(jnp.int32, (16, 1), 0)

    def h_row(i):
        q = (i // (2 * T)) * T + i % T
        return jnp.where((i // T) % 2 == 0, h0_v[pl.ds(q, 1), :], h1_v[pl.ds(q, 1), :])

    xs = jnp.where(row == 0, h_row(i1), jnp.where(row == 1, h_row(i2), 0.0))
    xs = _ln(xs).astype(BF16)
    cp_wg.wait()
    cp_wu.wait()
    cp_wd.wait()
    acts = []
    for j in range(wg_v.shape[0]):
        gate = _dot(xs, wg_v[j])
        up = _dot(xs, wu_v[j])
        acts.append((gate * jax.nn.sigmoid(gate) * up).astype(BF16))
    act = jnp.concatenate(acts, axis=1)
    y = jnp.concatenate([_dot(act, wd_v[j]) for j in range(G)], axis=1)
    y1 = y[0:1, :] * jax.nn.sigmoid(jnp.full((1, LANES), m1, F32))[:, 0:1]
    y2 = y[1:2, :] * jax.nn.sigmoid(jnp.full((1, LANES), m2, F32))[:, 0:1]

    b1 = pl.multiple_of((i1 // 16) * 16, 16)
    b2 = pl.multiple_of((i2 // 16) * 16, 16)

    def fixed(b):
        h2 = out_v[pl.ds(b, 16), :].astype(F32)
        t = row + b
        upd = jnp.where(t == i1, y1, 0.0) + jnp.where(t == i2, y2, 0.0)
        return (h2 + upd).astype(BF16)

    fix_v[0] = fixed(b1)
    fix_v[1] = fixed(b2)
    for i in range(nt):
        out_copy(i).wait()
    c1 = pltpu.make_async_copy(fix_v.at[0], out_hbm.at[pl.ds(b1, 16)], fix_sems.at[0])
    c2 = pltpu.make_async_copy(fix_v.at[1], out_hbm.at[pl.ds(b2, 16)], fix_sems.at[1])
    c1.start()

    @pl.when(b1 != b2)
    def _():
        c2.start()
        c2.wait()

    c1.wait()


@jax.jit
def pallas_sequential_preLN__linear_attn_block__moe_arch_mod__prompt_kernel(
        A_x, A_wqkv, A_wo, B_x, B_w_r, B_w_gate, B_w_up, B_w_down):
    del B_x
    B, S, D = A_x.shape
    Fd = B_w_gate.shape[1]
    nt = S // T
    any_spec = pl.BlockSpec(memory_space=pl.ANY)
    out = pl.pallas_call(
        _kernel,
        in_specs=[any_spec] * 7,
        out_specs=any_spec,
        out_shape=jax.ShapeDtypeStruct((S, D), A_x.dtype),
        scratch_shapes=[
            pltpu.VMEM((S, D), BF16),
            pltpu.VMEM((3, S, LANES), F32),
            pltpu.VMEM((8, 3 * D), F32),
            pltpu.VMEM((D, 3 * D), BF16),
            pltpu.VMEM((D, D), BF16),
            pltpu.VMEM((D,), BF16),
            pltpu.VMEM((Fd // LANES, D, LANES), BF16),
            pltpu.VMEM((Fd // LANES, D, LANES), BF16),
            pltpu.VMEM((D // LANES, Fd, LANES), BF16),
            pltpu.VMEM((D, S), BF16),
            pltpu.VMEM((D, D), BF16),
            pltpu.VMEM((2, 8, D), F32),
            pltpu.VMEM((D, D), BF16),
            pltpu.VMEM((2, D, LANES), F32),
            pltpu.VMEM((S, D), BF16),
            pltpu.VMEM((S, D), BF16),
            pltpu.VMEM((S // 2, D), F32),
            pltpu.VMEM((S // 2, D), F32),
            pltpu.VMEM((8, S // 8), F32),
            pltpu.VMEM((2, 16, D), BF16),
            pltpu.SemaphoreType.DMA((nt,)),
            pltpu.SemaphoreType.DMA((2 * D // NB1,)),
            pltpu.SemaphoreType.DMA((6,)),
            pltpu.SemaphoreType.DMA((nt,)),
            pltpu.SemaphoreType.DMA((2,)),
        ],
        compiler_params=pltpu.CompilerParams(vmem_limit_bytes=100 * 1024 * 1024),
    )(A_x.reshape(S, D), A_wqkv, A_wo, B_w_r, B_w_gate, B_w_up, B_w_down)
    return out.reshape(B, S, D)
```
